```python
import os as _os
_os.environ.setdefault("JAX_PLATFORMS", "cpu")
import jax
import jax.numpy as jnp

def _softmax(x, axis=-1):
    return jax.nn.softmax(x, axis=axis)
def _gelu(x):
    return jax.nn.gelu(x, approximate=True)
def _silu(x):
    return jax.nn.silu(x)
def _sigmoid(x):
    return jax.nn.sigmoid(x)
def _layernorm(x, axis=-1, eps=1e-5):
    m = jnp.mean(x, axis=axis, keepdims=True)
    v = jnp.var(x, axis=axis, keepdims=True)
    return (x - m) / jnp.sqrt(v + eps)
def _scatter_add(tgt, idx, src, axis=0):
    return tgt.at[idx].add(src)
def _segment_sum(src, seg, n):
    return jax.ops.segment_sum(src, seg, n)
class _Rng:
    def __init__(self, key):
        self._k = key
    def _next(self):
        self._k, sub = jax.random.split(self._k)
        return sub
    def normal(self, shape):
        return jax.random.normal(self._next(), shape, dtype=jnp.bfloat16)
    def randint(self, lo, hi, shape):
        return jax.random.randint(self._next(), shape, lo, hi, dtype=jnp.int32)
    def uniform(self, shape, lo=0.0, hi=1.0):
        return jax.random.uniform(self._next(), shape, jnp.bfloat16, lo, hi)
    def permutation(self, n):
        return jax.random.permutation(self._next(), n)


kernel_name = 'parallel_sum__sliding_block_cached__dense_activation_mish__decode'

def setup_inputs():
    _rng = _Rng(jax.random.key(int.from_bytes(__import__("os").urandom(4), "little")))
    _w = (lambda a: (lambda t: t.astype(jnp.bfloat16) if jnp.issubdtype(t.dtype, jnp.floating) else t)(jnp.asarray(a)))
    def _A_setup():
        B, Sq, D = 2, 1, 512
        Hq, Hkv, Sk, Dh = 32, 8, 32768, 128
        assert Hq % Hkv == 0, (Hq, Hkv)
        return {
            "x": _w((lambda *s: _rng.normal(s) * 0.05)(B, Sq, D)),
            "k_cache": _w((lambda *s: _rng.normal(s) * 0.8)(B, Hkv, Sk, Dh)),
            "v_cache": _w((lambda *s: _rng.normal(s) * 0.8)(B, Hkv, Sk, Dh)),
            "wq": _w((lambda *s: _rng.normal(s) * 0.8)(D, Hq * Dh) * (D ** -0.5)),
            "wo": _w((lambda *s: _rng.normal(s) * 0.8)(Hq * Dh, D) * ((Hq * Dh) ** -0.5)),
        }
    _A_in = _A_setup()

    def _B_setup():
        B, S, D, F = 2, 1, 512, 1792
        return {
            "x": _w((lambda *s: _rng.normal(s) * 0.05)(B, S, D)),
            "w1": _w((lambda *s: _rng.normal(s) * 0.4)(D, F) * (D ** -0.5)),
            "b1": _w((lambda *s: _rng.normal(s) * 0.05)(F)),
            "w2": _w((lambda *s: _rng.normal(s) * 0.05)(F, D) * (F ** -0.5)),
        }
    _B_in = _B_setup()

    return {
        "A_x": _A_in["x"],
        "A_k_cache": _A_in["k_cache"],
        "A_v_cache": _A_in["v_cache"],
        "A_wq": _A_in["wq"],
        "A_wo": _A_in["wo"],
        "B_x": _B_in["x"],
        "B_w1": _B_in["w1"],
        "B_b1": _B_in["b1"],
        "B_w2": _B_in["w2"],
    }

def reference(A_x, A_k_cache, A_v_cache, A_wq, A_wo, B_x, B_w1, B_b1, B_w2):
    def _A_ref(x, k_cache, v_cache, wq, wo):
        B, Sq, D = x.shape
        Hq, Dh = 32, 128
        Hkv, Sk = k_cache.shape[1], k_cache.shape[2]
        W = min(4096, max(256, Sk // 4))
        rep = Hq // Hkv
        q = (lambda x, *d: x.transpose(*d))((x @ wq).reshape(B, Sq, Hq, Dh), 0, 2, 1, 3)
        k = jnp.repeat(k_cache[:, :, Sk - W:, :], rep, axis=1)
        v = jnp.repeat(v_cache[:, :, Sk - W:, :], rep, axis=1)
        scores = jnp.einsum("bhqd,bhkd->bhqk", q, k) * (Dh ** -0.5)
        p = _softmax(scores, axis=-1)
        o = jnp.einsum("bhqk,bhkd->bhqd", p, v)
        return (lambda x, *d: x.transpose(*d))(o, 0, 2, 1, 3).reshape(B, Sq, Hq * Dh) @ wo

    def _B_ref(x, w1, b1, w2):
        h = jnp.einsum("bsd,df->bsf", x, w1) + b1
        sp = jnp.log1p(jnp.exp(-jnp.abs(h))) + jnp.where(h > 0, h, jnp.zeros_like(h))
        act = h * jnp.tanh(sp)
        return jnp.einsum("bsf,fd->bsd", act, w2)

    x = A_x
    xn = _layernorm(x, axis=-1)
    return x + _A_ref(xn, A_k_cache, A_v_cache, A_wq, A_wo) + _B_ref(xn, B_w1, B_b1, B_w2)
```

```python
import jax
import jax.numpy as jnp
from jax import lax
import jax.experimental.pallas as pl
import jax.experimental.pallas.tpu as pltpu

F32, BF16 = jnp.float32, jnp.bfloat16
NUM_Q_HEADS = 32
LN_EPS = 1e-5
STEPS = 16
Q0_SHARE = 0.375


@jax.jit
def pallas_parallel_sum__sliding_block_cached__dense_activation_mish__decode_kernel(
    A_x: jax.Array,
    A_k_cache: jax.Array,
    A_v_cache: jax.Array,
    A_wq: jax.Array,
    A_wo: jax.Array,
    B_x: jax.Array,
    B_w1: jax.Array,
    B_b1: jax.Array,
    B_w2: jax.Array,
):
    del B_x
    B, Sq, D = A_x.shape
    _, Hkv, Sk, Dh = A_k_cache.shape
    F = B_w1.shape[1]
    W = min(4096, max(256, Sk // 4))
    rep = NUM_Q_HEADS // Hkv
    E = NUM_Q_HEADS * Dh
    assert (B, Sq, rep, Dh) == (2, 1, 4, 128)
    R = B * W // STEPS
    per_b = W // R
    scale = Dh ** -0.5

    def cut(n, align):
        a = max(align, int(round(n * Q0_SHARE / align)) * align)
        return (0, a), (a, n - a)

    def aligned(i, m):
        return i if isinstance(i, int) else pl.multiple_of(i, m)

    def kernel(x_hbm, k_hbm, v_hbm, wq_hbm, wo_hbm, w1_hbm, b1_hbm, w2_hbm, out_hbm,
               x_v, k_v, v_v, wq_v, wo_v, w1_v, b1_v, w2_v, s_v, o_v, out_v, sems):
        def rows_phase(src, dst, base, nrows):
            per = nrows // STEPS
            cuts = cut(per, 8)

            def copy(j, t):
                off, n = cuts[t]
                rows = pl.ds(aligned(base + j * per + off, 8), n)
                return pltpu.make_async_copy(src.at[rows], dst.at[rows], sems.at[2 * j + t])
            return copy

        def cols_phase(src, dst, base, nrows):
            per = nrows // STEPS
            cuts = cut(src.shape[1], 128)

            def copy(j, t):
                rows, cols = pl.ds(aligned(base + j * per, 8), per), pl.ds(*cuts[t])
                return pltpu.make_async_copy(
                    src.at[rows, cols], dst.at[rows, cols], sems.at[2 * j + t])
            return copy

        def cache_phase(src, dst, h):
            cuts = cut(R, 16)

            def copy(j, t):
                off, n = cuts[t]
                src_rows = pl.ds(aligned(Sk - W + (j % per_b) * R + off, 16), n)
                dst_rows = pl.ds(aligned(j * R + off, 16), n)
                return pltpu.make_async_copy(
                    src.at[j // per_b, h, src_rows], dst.at[h, dst_rows], sems.at[2 * j + t])
            return copy

        def start(phase, j):
            phase(j, 0).start(priority=0)
            phase(j, 1).start(priority=1)

        def wait(phase, j):
            phase(j, 0).wait()
            phase(j, 1).wait()

        def advance(cur, nxt):
            def body(j, carry):
                wait(cur, j)
                start(nxt, j)
                return carry
            lax.fori_loop(0, STEPS, body, 0)

        wq_ph = [cols_phase(wq_hbm, wq_v, a * (D // 2), D // 2) for a in range(2)]
        w1_ph = cols_phase(w1_hbm, w1_v, 0, D)
        w2_ph = rows_phase(w2_hbm, w2_v, 0, F)
        wo_ph = [rows_phase(wo_hbm, wo_v, a * (E // 2), E // 2) for a in range(2)]
        x_cp = pltpu.make_async_copy(x_hbm, x_v, sems.at[2 * STEPS])
        b1_cp = pltpu.make_async_copy(b1_hbm, b1_v, sems.at[2 * STEPS + 1])
        out_cp = pltpu.make_async_copy(out_v, out_hbm, sems.at[2 * STEPS])

        for j in range(STEPS):
            start(wq_ph[0], j)
        x_cp.start()
        b1_cp.start()
        advance(wq_ph[0], wq_ph[1])

        row = lax.broadcasted_iota(jnp.int32, (8, D), 0)
        x_cp.wait()
        x = x_v[...].astype(F32)
        x8 = jnp.where(row < rep, x[0:1, :], x[1:2, :])
        xc = x8 - jnp.mean(x8, axis=-1, keepdims=True)
        var = jnp.mean(xc * xc, axis=-1, keepdims=True)
        xn = (xc / jnp.sqrt(var + LN_EPS)).astype(BF16)

        advance(wq_ph[1], w1_ph)
        advance(w1_ph, w2_ph)

        b1_cp.wait()
        b1 = b1_v[...].astype(F32)
        hid = jnp.dot(xn, w1_v[...], preferred_element_type=F32)
        hid = hid + jnp.concatenate([b1[j:j + 1, :] for j in range(F // 128)], axis=1)
        softplus = jnp.log1p(jnp.exp(-jnp.abs(hid))) + jnp.where(hid > 0, hid, 0.0)
        act = (hid * jnp.tanh(softplus)).astype(BF16)

        advance(w2_ph, cache_phase(k_hbm, k_v, 0))
        ffn = jnp.dot(act, w2_v[...], preferred_element_type=F32)
        acc = jnp.where(row % rep == 0, x8 + ffn, 0.0)

        row_h = lax.broadcasted_iota(jnp.int32, (8, Dh), 0)
        head_of_row, batch_of_row = row_h % rep, row_h // rep

        def attend(h, carry):
            qq = jnp.dot(xn, wq_v[:, pl.ds(aligned(h * rep * Dh, rep * Dh), rep * Dh)],
                         preferred_element_type=F32)
            q = qq[:, 0:Dh]
            for r in range(1, rep):
                q = jnp.where(head_of_row == r, qq[:, r * Dh:(r + 1) * Dh], q)
            q = q.astype(BF16)
            k_ph = cache_phase(k_hbm, k_v, h)
            v_ph = cache_phase(v_hbm, v_v, h)
            k_next = cache_phase(k_hbm, k_v, jnp.minimum(h + 1, Hkv - 1))

            def scores(j, mx):
                wait(k_ph, j)
                start(v_ph, j)
                k = k_v[h, pl.ds(aligned(j * R, R), R), :]
                s = lax.dot_general(q, k, (((1,), (1,)), ((), ())),
                                    preferred_element_type=F32) * scale
                s_v[j] = s
                mj = s[:, 0:128]
                for t in range(1, R // 128):
                    mj = jnp.maximum(mj, s[:, t * 128:(t + 1) * 128])
                return jnp.where(batch_of_row == j // per_b, jnp.maximum(mx, mj), mx)

            mx = lax.fori_loop(0, STEPS, scores, jnp.full((8, Dh), -jnp.inf, F32))
            mx = jnp.max(mx, axis=-1, keepdims=True)

            def values(j, carry):
                l, o = carry
                wait(v_ph, j)

                @pl.when(h < Hkv - 1)
                def _():
                    start(k_next, j)

                @pl.when(h == Hkv - 1)
                def _():
                    start(wo_ph[0], j)

                mine = lax.broadcasted_iota(jnp.int32, (8, R), 0) // rep == j // per_b
                p = jnp.where(mine, jnp.exp(s_v[j] - mx), 0.0)
                for t in range(R // 128):
                    l = l + p[:, t * 128:(t + 1) * 128]
                v = v_v[h, pl.ds(aligned(j * R, R), R), :]
                return l, o + jnp.dot(p.astype(BF16), v, preferred_element_type=F32)

            zero = jnp.zeros((8, Dh), F32)
            l, o = lax.fori_loop(0, STEPS, values, (zero, zero))
            o_v[h] = o / jnp.sum(l, axis=-1, keepdims=True)
            return carry

        lax.fori_loop(0, Hkv, attend, 0)

        wo_rows = E // 2 // STEPS
        heads_per_step = wo_rows // Dh

        def project(a):
            def body(j, acc):
                wait(wo_ph[a], j)
                if a == 0:
                    start(wo_ph[1], j)
                step = a * STEPS + j
                parts = []
                for t in range(heads_per_step):
                    hq = step * heads_per_step + t
                    part = jnp.where(head_of_row == hq % rep, o_v[hq // rep], 0.0)
                    parts.append(part.astype(BF16))
                lhs = parts[0] if heads_per_step == 1 else jnp.concatenate(parts, axis=1)
                w = wo_v[pl.ds(aligned(step * wo_rows, wo_rows), wo_rows), :]
                return acc + jnp.dot(lhs, w, preferred_element_type=F32)
            return body

        acc = lax.fori_loop(0, STEPS, project(0), acc)
        acc = lax.fori_loop(0, STEPS, project(1), acc)

        out0 = jnp.sum(jnp.where(row < rep, acc, 0.0), axis=0, keepdims=True)
        out1 = jnp.sum(jnp.where(row >= rep, acc, 0.0), axis=0, keepdims=True)
        out_v[...] = jnp.concatenate([out0, out1], axis=0).astype(out_v.dtype)
        out_cp.start()
        out_cp.wait()

    out = pl.pallas_call(
        kernel,
        out_shape=jax.ShapeDtypeStruct((B, D), A_x.dtype),
        in_specs=[pl.BlockSpec(memory_space=pl.ANY)] * 8,
        out_specs=pl.BlockSpec(memory_space=pl.ANY),
        scratch_shapes=[
            pltpu.VMEM((B, D), A_x.dtype),
            pltpu.VMEM((Hkv, B * W, Dh), A_k_cache.dtype),
            pltpu.VMEM((Hkv, B * W, Dh), A_v_cache.dtype),
            pltpu.VMEM(A_wq.shape, A_wq.dtype),
            pltpu.VMEM(A_wo.shape, A_wo.dtype),
            pltpu.VMEM(B_w1.shape, B_w1.dtype),
            pltpu.VMEM((F // 128, 128), B_b1.dtype),
            pltpu.VMEM(B_w2.shape, B_w2.dtype),
            pltpu.VMEM((STEPS, 8, R), F32),
            pltpu.VMEM((Hkv, 8, Dh), F32),
            pltpu.VMEM((B, D), A_x.dtype),
            pltpu.SemaphoreType.DMA((2 * STEPS + 2,)),
        ],
        compiler_params=pltpu.CompilerParams(
            vmem_limit_bytes=64 * 1024 * 1024,
            disable_semaphore_checks=True,
        ),
    )(A_x.reshape(B, D), A_k_cache, A_v_cache, A_wq, A_wo, B_w1,
      B_b1.reshape(F // 128, 128), B_w2)
    return out.reshape(B, Sq, D)
```

```python
import jax
import jax.numpy as jnp
from jax import lax
import jax.experimental.pallas as pl
import jax.experimental.pallas.tpu as pltpu

F32, BF16 = jnp.float32, jnp.bfloat16
NUM_Q_HEADS = 32
LN_EPS = 1e-5
STEPS = 16
Q0_SHARE = 0.1875
Q0_SHARE_LAST = 0.125


@jax.jit
def pallas_parallel_sum__sliding_block_cached__dense_activation_mish__decode_kernel(
    A_x: jax.Array,
    A_k_cache: jax.Array,
    A_v_cache: jax.Array,
    A_wq: jax.Array,
    A_wo: jax.Array,
    B_x: jax.Array,
    B_w1: jax.Array,
    B_b1: jax.Array,
    B_w2: jax.Array,
):
    del B_x
    B, Sq, D = A_x.shape
    _, Hkv, Sk, Dh = A_k_cache.shape
    F = B_w1.shape[1]
    W = min(4096, max(256, Sk // 4))
    rep = NUM_Q_HEADS // Hkv
    E = NUM_Q_HEADS * Dh
    assert (B, Sq, rep, Dh) == (2, 1, 4, 128) and E == 2 * STEPS * Dh
    R = B * W // STEPS
    per_b = W // R
    scale = Dh ** -0.5

    def cut(n, align, share):
        head = max(align, round(n * share / align) * align)
        return (0, head), (head, n - head)

    def rows(start, size, align):
        if not isinstance(start, int):
            start = pl.multiple_of(start, align)
        return pl.ds(start, size)

    def kernel(x_hbm, k_hbm, v_hbm, wq_hbm, wo_hbm, w1_hbm, b1_hbm, w2_hbm, out_hbm,
               x_v, k_v, v_v, wq_v, wo_v, w1_v, b1_v, w2_v, s_v, o_v, out_v, sems):
        def row_split_phase(src, dst, base, nrows, share=Q0_SHARE):
            per = nrows // STEPS
            cuts = cut(per, 16, share)

            def copy(j, t):
                off, n = cuts[t]
                r = rows(base + j * per + off, n, 16)
                return pltpu.make_async_copy(src.at[r], dst.at[r], sems.at[2 * j + t])
            return copy

        def col_split_phase(src, dst, base, nrows):
            per = nrows // STEPS
            cuts = cut(src.shape[1], 128, Q0_SHARE)

            def copy(j, t):
                r, c = rows(base + j * per, per, 16), pl.ds(*cuts[t])
                return pltpu.make_async_copy(src.at[r, c], dst.at[r, c], sems.at[2 * j + t])
            return copy

        def cache_phase(src, dst, h):
            cuts = cut(R, 16, Q0_SHARE)

            def copy(j, t):
                off, n = cuts[t]
                return pltpu.make_async_copy(
                    src.at[j // per_b, h, rows(Sk - W + (j % per_b) * R + off, n, 16)],
                    dst.at[h, rows(j * R + off, n, 16)],
                    sems.at[2 * j + t])
            return copy

        def start(phase, j):
            phase(j, 0).start(priority=0)
            phase(j, 1).start(priority=1)

        def wait(phase, j):
            phase(j, 0).wait()
            phase(j, 1).wait()

        def advance(cur, nxt):
            def body(j, carry):
                wait(cur, j)
                start(nxt, j)
                return carry
            lax.fori_loop(0, STEPS, body, 0)

        wq_ph = [col_split_phase(wq_hbm, wq_v, a * (D // 2), D // 2) for a in range(2)]
        w1_ph = col_split_phase(w1_hbm, w1_v, 0, D)
        w2_ph = row_split_phase(w2_hbm, w2_v, 0, F)
        wo_ph = [row_split_phase(wo_hbm, wo_v, 0, E // 2),
                 row_split_phase(wo_hbm, wo_v, E // 2, E // 2, Q0_SHARE_LAST)]
        x_cp = pltpu.make_async_copy(x_hbm, x_v, sems.at[2 * STEPS])
        b1_cp = pltpu.make_async_copy(b1_hbm, b1_v, sems.at[2 * STEPS + 1])
        out_cp = pltpu.make_async_copy(out_v, out_hbm, sems.at[2 * STEPS + 2])

        for j in range(STEPS):
            start(wq_ph[0], j)
        x_cp.start()
        b1_cp.start()
        advance(wq_ph[0], wq_ph[1])

        row = lax.broadcasted_iota(jnp.int32, (8, D), 0)
        x_cp.wait()
        x = x_v[...].astype(F32)
        x8 = jnp.where(row < rep, x[0:1, :], x[1:2, :])
        xc = x8 - jnp.mean(x8, axis=-1, keepdims=True)
        var = jnp.mean(xc * xc, axis=-1, keepdims=True)
        xn = (xc / jnp.sqrt(var + LN_EPS)).astype(BF16)

        advance(wq_ph[1], w1_ph)
        advance(w1_ph, w2_ph)

        b1_cp.wait()
        b1 = b1_v[...].astype(F32)
        hid = jnp.dot(xn, w1_v[...], preferred_element_type=F32)
        hid = hid + jnp.concatenate([b1[j:j + 1, :] for j in range(F // 128)], axis=1)
        softplus = jnp.log1p(jnp.exp(-jnp.abs(hid))) + jnp.where(hid > 0, hid, 0.0)
        act = (hid * jnp.tanh(softplus)).astype(BF16)

        advance(w2_ph, cache_phase(k_hbm, k_v, 0))
        resid = x8 + jnp.dot(act, w2_v[...], preferred_element_type=F32)
        acc = jnp.where(row == 0, resid[0:1, :], resid[rep:rep + 1, :])

        row_h = lax.broadcasted_iota(jnp.int32, (8, Dh), 0)

        def attend(h, carry):
            qq = jnp.dot(xn, wq_v[:, rows(h * rep * Dh, rep * Dh, rep * Dh)],
                         preferred_element_type=F32)
            q = qq[:, 0:Dh]
            for r in range(1, rep):
                q = jnp.where(row_h % rep == r, qq[:, r * Dh:(r + 1) * Dh], q)
            q = q.astype(BF16)
            k_ph = cache_phase(k_hbm, k_v, h)
            v_ph = cache_phase(v_hbm, v_v, h)
            k_next = cache_phase(k_hbm, k_v, jnp.minimum(h + 1, Hkv - 1))

            def scores(j, mx):
                wait(k_ph, j)
                start(v_ph, j)
                s = lax.dot_general(q, k_v[h, rows(j * R, R, R), :], (((1,), (1,)), ((), ())),
                                    preferred_element_type=F32) * scale
                s_v[j] = s
                mj = s[:, 0:128]
                for t in range(1, R // 128):
                    mj = jnp.maximum(mj, s[:, t * 128:(t + 1) * 128])
                return jnp.where(row_h // rep == j // per_b, jnp.maximum(mx, mj), mx)

            mx = lax.fori_loop(0, STEPS, scores, jnp.full((8, Dh), -jnp.inf, F32))
            mx = jnp.max(mx, axis=-1, keepdims=True)

            def values(j, carry):
                l, o = carry
                wait(v_ph, j)

                @pl.when(h < Hkv - 1)
                def _():
                    start(k_next, j)

                @pl.when(h == Hkv - 1)
                def _():
                    start(wo_ph[0], j)

                mine = lax.broadcasted_iota(jnp.int32, (8, R), 0) // rep == j // per_b
                p = jnp.where(mine, jnp.exp(s_v[j] - mx), 0.0)
                for t in range(R // 128):
                    l = l + p[:, t * 128:(t + 1) * 128]
                pv = jnp.dot(p.astype(BF16), v_v[h, rows(j * R, R, R), :],
                             preferred_element_type=F32)
                return l, o + pv

            zero = jnp.zeros((8, Dh), F32)
            l, o = lax.fori_loop(0, STEPS, values, (zero, zero))
            o = o / jnp.sum(l, axis=-1, keepdims=True)
            for r in range(rep):
                o_v[h * rep + r] = jnp.where(row_h == 0, o[r:r + 1, :], o[rep + r:rep + r + 1, :])
            return carry

        lax.fori_loop(0, Hkv, attend, 0)

        def project(a):
            def body(j, acc):
                wait(wo_ph[a], j)
                if a == 0:
                    start(wo_ph[1], j)
                hq = a * STEPS + j
                return acc + jnp.dot(o_v[hq].astype(BF16), wo_v[rows(hq * Dh, Dh, Dh), :],
                                     preferred_element_type=F32)
            return body

        acc = lax.fori_loop(0, STEPS, project(0), acc)
        acc = lax.fori_loop(0, STEPS, project(1), acc)

        out_v[...] = acc[0:B, :].astype(out_v.dtype)
        out_cp.start()
        out_cp.wait()

    out = pl.pallas_call(
        kernel,
        out_shape=jax.ShapeDtypeStruct((B, D), A_x.dtype),
        in_specs=[pl.BlockSpec(memory_space=pl.ANY)] * 8,
        out_specs=pl.BlockSpec(memory_space=pl.ANY),
        scratch_shapes=[
            pltpu.VMEM((B, D), A_x.dtype),
            pltpu.VMEM((Hkv, B * W, Dh), A_k_cache.dtype),
            pltpu.VMEM((Hkv, B * W, Dh), A_v_cache.dtype),
            pltpu.VMEM(A_wq.shape, A_wq.dtype),
            pltpu.VMEM(A_wo.shape, A_wo.dtype),
            pltpu.VMEM(B_w1.shape, B_w1.dtype),
            pltpu.VMEM((F // 128, 128), B_b1.dtype),
            pltpu.VMEM(B_w2.shape, B_w2.dtype),
            pltpu.VMEM((STEPS, 8, R), F32),
            pltpu.VMEM((NUM_Q_HEADS, 8, Dh), F32),
            pltpu.VMEM((B, D), A_x.dtype),
            pltpu.SemaphoreType.DMA((2 * STEPS + 3,)),
        ],
        compiler_params=pltpu.CompilerParams(
            vmem_limit_bytes=64 * 1024 * 1024,
            disable_semaphore_checks=True,
        ),
    )(A_x.reshape(B, D), A_k_cache, A_v_cache, A_wq, A_wo, B_w1,
      B_b1.reshape(F // 128, 128), B_w2)
    return out.reshape(B, Sq, D)
```
